```python
import os as _os
_os.environ.setdefault("JAX_PLATFORMS", "cpu")
import jax
import jax.numpy as jnp

def _softmax(x, axis=-1):
    return jax.nn.softmax(x, axis=axis)
def _gelu(x):
    return jax.nn.gelu(x, approximate=True)
def _silu(x):
    return jax.nn.silu(x)
def _sigmoid(x):
    return jax.nn.sigmoid(x)
def _layernorm(x, axis=-1, eps=1e-5):
    m = jnp.mean(x, axis=axis, keepdims=True)
    v = jnp.var(x, axis=axis, keepdims=True)
    return (x - m) / jnp.sqrt(v + eps)
def _scatter_add(tgt, idx, src, axis=0):
    return tgt.at[idx].add(src)
def _segment_sum(src, seg, n):
    return jax.ops.segment_sum(src, seg, n)
class _Rng:
    def __init__(self, key):
        self._k = key
    def _next(self):
        self._k, sub = jax.random.split(self._k)
        return sub
    def normal(self, shape):
        return jax.random.normal(self._next(), shape, dtype=jnp.bfloat16)
    def randint(self, lo, hi, shape):
        return jax.random.randint(self._next(), shape, lo, hi, dtype=jnp.int32)
    def uniform(self, shape, lo=0.0, hi=1.0):
        return jax.random.uniform(self._next(), shape, jnp.bfloat16, lo, hi)
    def permutation(self, n):
        return jax.random.permutation(self._next(), n)


kernel_name = 'interleave_layers__linear_kernel_hedgehog__sliding_block__prompt'

def setup_inputs():
    _rng = _Rng(jax.random.key(int.from_bytes(__import__("os").urandom(4), "little")))
    _w = (lambda a: (lambda t: t.astype(jnp.bfloat16) if jnp.issubdtype(t.dtype, jnp.floating) else t)(jnp.asarray(a)))
    def _A_setup():
        B, S, D, H = 1, 2048, 448, 16
        Dh = D // H
        return {
            "x": _w((lambda *s: _rng.normal(s) * 0.05)(B, S, D)),
            "wqkv": _w((lambda *s: _rng.normal(s) * 0.4)(D, 3 * D)),
            "w_phi": _w((lambda *s: _rng.normal(s) * 0.4)(H, Dh, Dh) * (Dh ** -0.5)),
            "wo": _w((lambda *s: _rng.normal(s) * 0.05)(D, D)),
        }
    _A_in = _A_setup()

    def _B_setup():
        B, S, D = 1, 2048, 448
        return {
            "x": _w((lambda *s: _rng.normal(s) * 0.05)(B, S, D)),
            "wqkv": _w((lambda *s: _rng.normal(s) * 0.1)(D, 3 * D)),
            "wo": _w((lambda *s: _rng.normal(s) * 0.1)(D, D)),
        }
    _B_in = _B_setup()

    return {
        "A_x": _A_in["x"],
        "A_wqkv": _A_in["wqkv"],
        "A_w_phi": _A_in["w_phi"],
        "A_wo": _A_in["wo"],
        "B_x": _B_in["x"],
        "B_wqkv": _B_in["wqkv"],
        "B_wo": _B_in["wo"],
    }

def reference(A_x, A_wqkv, A_w_phi, A_wo, B_x, B_wqkv, B_wo):
    def _A_ref(x, wqkv, w_phi, wo):
        B, S, D = x.shape
        H = 16; Dh = D // H
        qkv = (lambda x, *d: x.transpose(*d))((x @ wqkv).reshape(B, S, 3, H, Dh), 2, 0, 3, 1, 4)
        q, k, v = qkv[0], qkv[1], qkv[2]
        pq = jnp.einsum("bhsd,hdf->bhsf", q, w_phi)
        pk = jnp.einsum("bhsd,hdf->bhsf", k, w_phi)
        phi_q = jnp.concatenate([_softmax(pq, axis=-1), _softmax(-pq, axis=-1)], axis=-1)
        phi_k = jnp.concatenate([_softmax(pk, axis=-1), _softmax(-pk, axis=-1)], axis=-1)
        kv = jnp.einsum("bhsf,bhsd->bhfd", phi_k, v)
        z  = jnp.einsum("bhsf->bhf", phi_k)
        num = jnp.einsum("bhqf,bhfd->bhqd", phi_q, kv)
        den = jnp.einsum("bhqf,bhf->bhq", phi_q, z)[..., None] + 1e-6
        o = num / den
        return (lambda x, *d: x.transpose(*d))(o, 0, 2, 1, 3).reshape(B, S, D) @ wo

    def _B_ref(x, wqkv, wo):
        B, S, D = x.shape
        H = 16; Dh = D // H; W = 256
        qkv = (lambda x, *d: x.transpose(*d))((x @ wqkv).reshape(B, S, 3, H, Dh), 2, 0, 3, 1, 4)
        q, k, v = qkv[0], qkv[1], qkv[2]
        scores = jnp.einsum("bhqd,bhkd->bhqk", q, k) * (Dh ** -0.5)
        idx = jnp.arange(S)
        mask = (idx[:, None] - idx[None, :] >= 0) & (idx[:, None] - idx[None, :] < W)
        scores = jnp.where(mask[None, None], scores, -1e9)
        p = _softmax(scores, axis=-1)
        o = jnp.einsum("bhqk,bhkd->bhqd", p, v)
        return (lambda x, *d: x.transpose(*d))(o, 0, 2, 1, 3).reshape(B, S, D) @ wo

    x = A_x
    x = x + _A_ref(_layernorm(x, axis=-1), A_wqkv, A_w_phi, A_wo)
    x = x + _B_ref(_layernorm(x, axis=-1), B_wqkv, B_wo)
    x = x + _A_ref(_layernorm(x, axis=-1), A_wqkv, A_w_phi, A_wo)
    x = x + _B_ref(_layernorm(x, axis=-1), B_wqkv, B_wo)
    return x
```

```python
import jax
import jax.numpy as jnp
import numpy as np
import jax.experimental.pallas as pl
import jax.experimental.pallas.tpu as pltpu

S, D, H, DH, WIN = 2048, 448, 16, 28, 256
T = 256
NCH = S // T
UNITS = 4 * (T // 128)
NBUF = 4
MH, KH = D // 2, 256
LEFT, RIGHT = "left", "right"
DEFAULT = (0, 0.0, 0.6, 0.4, 0.9, 0.0, 1.0, 0, 0)
TUNING = {
    (0, 0): (4, 0.2, 0.6, 0.4, 0.7, 0.2, 0.8, 0, 0),
    (0, 1): (2, 0, 0.6, 0.6, 0.9, 0.2, 0.8, 0, 1),
    (0, 2): (0, 0.2, 1.0, 0, 0.9, 0, 1.0, 0, 0),
    (0, 3): (0, 0.2, 0.6, 0.4, 0.9, 0.0, 0.8, 1, 0),
    (0, 4): (4, 0, 0.6, 0.4, 0.9, 0, 1.0, 0, 0),
    (0, 5): (5, 0, 0.8, 0.6, 0.7, 0.2, 0.6, 0, 0),
    (0, 6): (0, 0.1, 0.4, 0.2, 0.8, 0.2, 1.0, 0, 0),
    (0, 7): (2, 0.0, 0.8, 0, 1.0, 0.2, 1.0, 1, 0),
    (1, -1): (2, 0.2, 0.8, 0.2, 0.9, 0, 0.8, 0, 1),
    (1, 0): (3, 0, 0.6, 0, 0.7, 0.2, 1.0, 1, 0),
    (1, 1): (5, 0, 0.8, 0, 0.8, 0.0, 0.8, 0, 0),
    (1, 2): (3, 0, 0.4, 0.4, 1.0, 0, 1.0, 0, 1),
    (1, 3): (3, 0, 0.6, 0.2, 0.9, 0.2, 1.0, 0, 0),
    (1, 4): (3, 0.0, 0.4, 0.4, 1.0, 0.2, 1.0, 0, 0),
    (1, 5): (1, 0.0, 0.6, 0.6, 0.9, 0, 0.8, 1, 1),
    (1, 6): (1, 0.0, 0.4, 0.4, 1.0, 0, 0.6, 0, 1),
    (1, 7): (4, 0, 1.0, 0.2, 0.7, 0, 1.0, 0, 0),
    (1, 8): (0, 0, 1.0, 0, 0.7, 0.2, 1.0, 0, 1),
    (2, -1): (0, 0.2, 0.4, 0.2, 0.9, 0.2, 0.6, 0, 0),
    (2, 0): (0, 0, 0.4, 0.2, 0.7, 0.2, 1.0, 0, 0),
    (2, 1): (4, 0, 0.4, 0.4, 1.0, 0.2, 0.8, 1, 0),
    (2, 2): (5, 0.2, 1.0, 0.4, 0.9, 0, 1.0, 0, 0),
    (2, 3): (2, 0.1, 0.8, 0, 0.7, 0, 1.0, 0, 1),
    (2, 4): (1, 0, 0.4, 0.4, 1.0, 0, 0.8, 0, 1),
    (2, 5): (1, 0, 1.0, 0, 0.9, 0, 1.0, 0, 0),
    (2, 6): (4, 0.2, 0.8, 0.2, 0.9, 0.2, 0.6, 1, 1),
    (2, 7): (2, 0.1, 1.0, 0.2, 0.7, 0, 1.0, 1, 1),
    (2, 8): (1, 0.1, 1.0, 0.2, 0.9, 0.0, 1.0, 0, 1),
}
LOG2E = float(np.log2(np.e))
F32, BF16, U32 = jnp.float32, jnp.bfloat16, jnp.uint32
NN = (((1,), (0,)), ((), ()))
NT = (((1,), (1,)), ((), ()))


def _dot(a, b, dims=NN):
    return jax.lax.dot_general(a, b, dims, preferred_element_type=F32)


def _iota(shape, dim):
    return jax.lax.broadcasted_iota(jnp.int32, shape, dim)


def _tree(op, xs):
    xs = list(xs)
    while len(xs) > 1:
        xs = [op(xs[i], xs[i + 1]) if i + 1 < len(xs) else xs[i] for i in range(0, len(xs), 2)]
    return xs[0]


def _chain(op, xs, ways=1):
    acc = list(xs[:ways])
    for i, x in enumerate(xs[ways:]):
        acc[i % ways] = op(acc[i % ways], x)
    return _tree(op, acc)


def _rows8(x):
    return [x[i:i + 8] for i in range(0, x.shape[0], 8)]


def _allsub(op, x, shifts=(4, 2, 1)):
    for s in shifts:
        x = op(x, pltpu.roll(x, s, 0))
    return x


def _recip(x):
    r = pl.reciprocal(x, approx=True)
    return r * (2.0 - x * r)


def _words(ref):
    return ref.bitcast(U32)


def _put(ref, i, x, row=0):
    for j in range(2):
        ref[i, j, row:row + x.shape[0], :] = x[:, 128 * j:128 * j + 128]


def _get(ref, i):
    return jnp.concatenate([_words(ref)[i, j] for j in range(2)], axis=1)


def _halves(x):
    return pltpu.bitcast(x, BF16)


def _operands(block, dst):
    for r in range(0, KH, 16):
        top = block(r)
        b11, b12 = top[:, 0:128], top[:, 128:256]
        if KH + r < D:
            bot = block(KH + r)
            b21, b22 = bot[:, 0:128], bot[:, 128:256]
            ops = [b11, b21 - b11, b12 - b22, b22, b11 + b22, b21 + b22, b11 + b12]
        else:
            ops = [b11, -b11, b12, None, b11, None, b11 + b12]
        for i, v in enumerate(ops):
            if v is not None:
                dst[i, r:r + 16, :] = v.astype(BF16)


def _layernorm(rows, reload, dst):
    shift = _allsub(jnp.add, rows[0]) * 0.125
    dev = [r - shift for r in rows]
    off = _allsub(jnp.add, _chain(jnp.add, dev)) * (1.0 / D)
    var = _allsub(jnp.add, _chain(jnp.add, [d * d for d in dev])) * (1.0 / D)
    var = jnp.maximum(var - off * off, 0.0)
    mean = shift + off
    rstd = jax.lax.rsqrt(var + 1e-5)
    mean, rstd = (jnp.concatenate([v] * 2, axis=0) for v in (mean, rstd))
    _operands(lambda r: (reload(r) - mean) * rstd, dst)


def _feature_map(p):
    rows = _rows8(p)
    hi = _allsub(jnp.maximum, _chain(jnp.maximum, rows), (4, 2))
    lo = _allsub(jnp.minimum, _chain(jnp.minimum, rows), (4, 2))
    out = []
    for e in ([jnp.exp2(r - hi) for r in rows], [jnp.exp2(lo - r) for r in rows]):
        inv = _recip(_allsub(jnp.add, _chain(jnp.add, e, 2), (4, 2)))
        out += [v * inv for v in e]
    out.append(jnp.zeros((16, p.shape[1]), F32))
    return jnp.concatenate(out, axis=0).astype(BF16)


def _kernel(x_hbm, awqkv_hbm, wphi_hbm, awo_hbm, bwqkv_hbm, bwo_hbm, o_hbm,
            xin, wraw_a, wraw_b, woraw_a, woraw_b, wphi, wa, wb, woa, wob,
            wtmp, phiq, kvmat, kn, vt, qs, phik, av, ao, bo, obuf, sem_x, sem_w, sem_o, slot, tbuf, pbuf, sbuf, xres, an, bn):
    def tok(c):
        return slice(c * T, (c + 1) * T)

    x_copies = [pltpu.make_async_copy(x_hbm.at[:, tok(c)], xin[c].at[0], sem_x.at[c])
                for c in range(NCH)]
    o_copies = [pltpu.make_async_copy(obuf.at[:, tok(c)], o_hbm.at[:, tok(c)], sem_o.at[c])
                for c in range(NCH)]
    w_copies = [pltpu.make_async_copy(s, d, sem_w.at[i]) for i, (s, d) in enumerate(
        [(awqkv_hbm.at[:, 2 * D:], wraw_a.at[:, 2 * D:]), (wphi_hbm, wphi),
         (awqkv_hbm.at[:, 384:2 * D], wraw_a.at[:, 384:2 * D]),
         (awqkv_hbm.at[:, :384], wraw_a.at[:, :384]), (awo_hbm, woraw_a),
         (bwqkv_hbm, wraw_b), (bwo_hbm, woraw_b)])]
    zeros = [pl.semaphore_read(slot.at[i]) for i in range(3)]
    for cp in (w_copies[1], x_copies[0], w_copies[0], w_copies[2]):
        cp.start()

    low = _iota((8, 128), 0) < 4
    lowt = _iota((8, T), 0) < 4
    val = {}

    def fold_matrices():
        wp = wphi[...].reshape(DH * H, DH)
        r, c = _iota((D, D), 0), _iota((D, D), 1)
        perm = jnp.where((c & 15) * DH + (c >> 4) == r, 1.0, 0.0).astype(BF16)
        wp = _dot(perm, wp).astype(BF16)
        r, c = _iota((112, DH), 0), _iota((112, DH), 1)
        pick = jnp.where((jnp.where(r >= 56, r - 56, r) >> 1) == c, 1.0, 0.0).astype(BF16)
        r, c = _iota((112, 112), 0), _iota((112, 112), 1)
        head = jnp.where(r >= 56, 2, 0) + (r & 1)
        same = (c >= head * DH) & (c < head * DH + DH)
        return [jnp.where(same, _dot(pick, wp[112 * g:112 * g + 112], NT), 0.0).astype(BF16)
                for g in range(4)]

    def transpose(dst, src, blocks):
        for j in blocks:
            cols = slice(128 * j, min(src.shape[1], 128 * j + 128))
            for t in range(4):
                v = src[128 * t:min(D, 128 * t + 128), cols]
                if t == 3:
                    v = jnp.concatenate([v, jnp.zeros((2 * KH - D, v.shape[1]), BF16)], axis=0)
                n = src.shape[1]
                dst[0, t * n + cols.start:t * n + cols.stop, :] = v.astype(F32).T.astype(BF16)

    def weight_rows(src, r, size):
        n = src.shape[1] // 4
        return _halves(jnp.concatenate([_words(src)[0, (t * n + r) // 2:(t * n + r + size) // 2, :]
                                        for t in range(4)], axis=1))

    def prepare(dst, part, src, scale=None):
        def block(r):
            if r < MH:
                pace(src, r / MH)
            v = weight_rows(src, part * D + r, 16).astype(F32)
            return v if scale is None else v * scale
        combine(dst, part, block)

    def combine(dst, part, block):
        for r in range(0, MH, 16):
            top, bot = block(r), block(MH + r)
            a11, a21 = top[:, 0:KH], bot[:, 0:KH]
            a12, a22 = top[:, KH:], bot[:, KH:]
            for i, v in enumerate([a21 + a22, a22, a11, a11 + a12, a11 + a22, a12 - a22, a21 - a11]):
                _put(dst, 7 * part + i, v.astype(BF16), r)

    def project(w, part, src):
        def mul(i):
            return _dot(_halves(_get(w, 7 * part + i)), _halves(_words(src)[i]))
        m2, m4, m3, m5 = mul(0), mul(1), mul(2), mul(3)
        ticks = val["ticks"] = _rows8(m4) + _rows8(m5)
        whole = yield
        m1, m7, m6 = mul(4), mul(5), mul(6)
        val["ticks"] = (ticks if whole else []) + _rows8(m7) + _rows8(m6)[:MH // 16]
        top = jnp.concatenate([(m4 - m5) + m1 + m7, m3 + m5], axis=1)
        bot = jnp.concatenate([m2 + m4, (m3 - m2) + m1 + m6], axis=1)
        return jnp.concatenate([top, bot], axis=0)

    def fold_into(fold, part):
        y = [_dot(fold[g], weight_rows(wtmp[0], part * D + 112 * g, 112)) * LOG2E
             for g in range(4)]
        y = jnp.concatenate(y, axis=0)
        combine(wa, part, lambda r: y[r:r + 16])

    def span(i, frac):
        start, end = val["tune"][i:i + 2]
        return start + (end - start) * frac

    def pace(ref, frac):
        ticks = val.get("ticks")
        if ticks:
            tick = ticks[min(int(frac * len(ticks)), len(ticks) - 1)]
            if ref.dtype == BF16 and ref.shape[-1] != 128:
                tick = jnp.concatenate([tick, tick], axis=0).astype(BF16)
            elif ref.dtype == BF16:
                ref, tick = _words(ref), pltpu.bitcast(tick, U32)
            ref[zeros[0] + 1, 0:tick.shape[0], 0:128] = tick

    def a_norm(c):
        def load(r):
            if r < KH:
                pace(xin[c], span(5, r / KH))
            return xin[c][zeros[1], r:r + 16, :].astype(F32)
        _layernorm(_rows8(xin[c][0].astype(F32)), load, an[c])

    def residual(c, x, dst):
        def load(r):
            if r < KH:
                pace(xres[c], span(5, r / KH))
            return xres[c][zeros[1], r:r + 16, :]
        xres[c][0] = x
        rows = _rows8(x)
        rows = [jnp.concatenate([rows[(r + MH // 8) % (D // 8)][:, 0:128], rows[r][:, 128:256]], axis=1)
                for r in range(D // 8)]
        while val["tune"][7] and val.get("short"):
            yield
        _layernorm(rows, load, dst)

    def features(y, dst):
        yield
        for p in range(8):
            _put(dst, p, _feature_map(y[56 * p:56 * p + 56]))

    def a_q(c):
        y = (yield from project(wa, 0, an[c]))
        yield from features(y, phiq[c % 2])

    def a_k(c):
        y = (yield from project(wa, 1, an[c]))
        yield from features(y, phik[c % 2])

    def a_v(c):
        y = (yield from project(wa, 2, an[c]))
        yield
        ones = jnp.ones((8, T), F32)
        for p in range(8):
            _put(av[c % 2], p, jnp.concatenate([y[56 * p:56 * p + 56], ones], axis=0).astype(BF16))

    def a_kv(c):
        kv = [_dot(_halves(_get(av[c % 2], p)), _halves(_get(phik[c % 2], p)), NT) for p in range(8)]
        val["kv"] = kv if c == 0 else [a + b for a, b in zip(val["kv"], kv)]
        if c == NCH - 1:
            r, l = _iota((64, 128), 0), _iota((64, 128), 1)
            keep = (((r >= DH) & (r < 56)) | (r >= 60)) == ((l & 1) == 1)
            for p in range(8):
                kvmat[p] = jnp.where(keep, val["kv"][p], 0.0).astype(BF16)

    def a_num(c):
        out = []
        nums = [_dot(_halves(_words(kvmat)[p]), _halves(_get(phiq[c % 2], p))) for p in range(8)]
        yield
        for p in range(8):
            rows = _rows8(nums[p])
            inv = _recip(rows[7] + 1e-6)
            swp = pltpu.roll(inv, 4, 0)
            i0, i1 = jnp.where(lowt, inv, swp), jnp.where(lowt, swp, inv)
            out += [v * i0 for v in rows[0:3]] + [rows[3] * inv] + [v * i1 for v in rows[4:7]]
        _operands(lambda r: jnp.concatenate(out[r // 8:r // 8 + 2], axis=0), ao[c % 2])

    def a_out(c):
        y = yield from project(woa, 0, ao[c % 2])
        x = (xin[c][zeros[2]].astype(F32) if val["first"] else xres[c][0]) + y
        yield
        yield from residual(c, x, bn[c % 2])

    def spin(rows, sign):
        def rot(v, c):
            return pltpu.roll(v, (sign * 32 * c) % 128, 1)
        return (rows[0:3] + [jnp.where(low, rows[3], rot(rows[3], 1))]
                + [rot(v, 1) for v in rows[4:7]] + [rot(v, 2) for v in rows[7:10]]
                + [jnp.where(low, rot(rows[10], 2), rot(rows[10], 3))]
                + [rot(v, 3) for v in rows[11:14]])

    def b_q(c):
        y = (yield from project(wb, 0, bn[c % 2]))
        yield
        for u in range(UNITS):
            i, g = divmod(u, 4)
            q = y[112 * g:112 * g + 112, 128 * i:128 * i + 128]
            qs[c % 2, u] = jnp.concatenate(spin(_rows8(q), 1), axis=0).astype(BF16)

    def b_k(c):
        y = (yield from project(wb, 1, bn[c % 2]))
        yield
        for g in range(4):
            k = jnp.concatenate([y[112 * g:112 * g + 112], jnp.zeros((16, y.shape[1]), F32)], axis=0)
            kn[g, tok(c), :] = k.T.astype(BF16)

    def b_v(c):
        y = (yield from project(wb, 2, bn[c % 2]))
        yield
        for p in range(8):
            v = _rows8(y[56 * p:56 * p + 56])
            half = _iota(v[3].shape, 0) < 4
            v = v[0:3] + [jnp.where(half, v[3], 1.0), jnp.where(half, 1.0, v[3])] + v[4:7]
            v = jnp.concatenate(v, axis=0).astype(BF16)
            for i in range(T // 128):
                vt[c * T // 128 + i, 64 * p:64 * p + 64, :] = v[:, 128 * i:128 * i + 128]

    def b_scores(c, u):
        i, g = divmod(u, 4)
        base = c * T + 128 * i
        q = _words(qs)[c % 2, u]
        r, l = _iota((56, 128), 0), _iota((56, 128), 1)
        head = ((r >= 14).astype(jnp.int32) + (r >= 28).astype(jnp.int32)
                + (r >= 42).astype(jnp.int32))
        tile = ((l >> 5) - head) & 3
        far = _iota((32, 128), 0) > (_iota((32, 128), 1) & 31)
        tops, ticks = [], []
        n_unit = c * UNITS + u
        prev = b_pv(*divmod(n_unit - 2, UNITS)) if n_unit >= 2 else iter(())
        for j in range(4):
            rhs = jnp.concatenate([jnp.where(tile == j, q, jnp.zeros_like(q)),
                                   jnp.zeros((8, 128), U32)], axis=0)
            lo, hi = base + 32 * j - WIN, base + 32 * j + 32
            s = _dot(_halves(_words(kn)[g, max(lo, 0) // 2:hi // 2, :]), _halves(rhs))
            n = s.shape[0]
            ticks = _rows8(s)
            rows = _rows8(s[(32 if lo >= 0 else 0):n - 32]) if n > 32 else []
            rows += _rows8(jnp.where(far, s[0:32] if lo >= 0 else -1e30, s[n - 32:n]))
            if val["tune"][8]:
                sbuf[4 * (u % NBUF) + j][0, 0:8 * len(rows), :] = jnp.concatenate(rows, axis=0)
            tops.append((_allsub(jnp.maximum, _chain(jnp.maximum, rows)), rows))
        val["top", c, u] = tops, val["tune"][8]
        next(prev, None)
        val["ticks"] = ticks
        yield
        next(prev, None)
        b_probs(c, u)
        if n_unit >= 1:
            b_mix(*divmod(n_unit - 1, UNITS))

    def b_probs(c, u):
        base = c * T + 128 * (u // 4)
        far = _iota((32, 128), 0) > (_iota((32, 128), 1) & 31)
        tops, staged = val["top", c, u]
        for j, (top, rows) in enumerate(tops):
            if staged:
                rows = [sbuf[4 * (u % NBUF) + j][zeros[0], 8 * r:8 * r + 8, :] for r in range(len(rows))]
            tbuf[u % NBUF][0, 8 * j:8 * j + 8, :] = top
            pace(tbuf[u % NBUF], span(1, j / 4))
            top = tbuf[u % NBUF][zeros[1], 8 * j:8 * j + 8, :]
            e = [jnp.exp2(v - top) for v in rows]
            if base + 32 * j >= WIN:
                edge = jnp.concatenate(e[-4:], axis=0)
                e = [jnp.where(far, edge, 0.0)] + e[:-4] + [jnp.where(far, 0.0, edge)]
            e = jnp.concatenate(e, axis=0).astype(BF16)
            pbuf[u % NBUF][0, 288 * j + 288 - e.shape[0]:288 * j + 288, :] = e

    def b_mix(c, u):
        base = c * T + 128 * (u // 4)
        zero = jnp.zeros((16, 128), jnp.uint32)

        def mix(mask, a, b):
            if a is None and b is None:
                return None
            return jnp.where(mask, zero if a is None else a, zero if b is None else b)

        grp = _iota((16, 128), 1) >> 5
        odd, upper = (grp & 1) == 1, grp >= 2
        first = max(WIN - base, 0)
        for k in range(first, 384, 32):
            pace(pbuf[u % NBUF], span(3, k / 384))
            xs = [_words(pbuf[u % NBUF])[0, 128 * j + k // 2:128 * j + k // 2 + 16, :]
                  if 0 <= k - 32 * j < 288 else None for j in range(4)]
            ys = [mix(odd, xs[(a + 1) % 4], xs[a]) for a in range(4)]
            for h in range(4):
                val["p", c, u, h, k - first] = mix(upper, ys[(2 - h) % 4], ys[(-h) % 4])

    def b_pv(c, u):
        i, g = divmod(u, 4)
        base = c * T + 128 * i
        lo = max(base - WIN, 0)
        acc = [None] * 4
        for t in range((base + 128 - lo) // 128):
            for h in range(4):
                p = jnp.concatenate([val["p", c, u, h, 128 * t + k] for k in range(0, 128, 32)], axis=0)
                rows = slice(16 * (4 * g + h), 16 * (4 * g + h + 1))
                o = _dot(_halves(_words(vt)[lo // 128 + t, rows, :]), _halves(p))
                acc[h] = o if t == 0 else acc[h] + o
        acc = [_rows8(o) for o in acc]
        yield
        out = []
        for a, b in (acc[0:2], acc[2:4]):
            inv = _recip(jnp.where(low, b[0], a[3]))
            swp = pltpu.roll(inv, 4, 0)
            i0, i1 = jnp.where(low, swp, inv), jnp.where(low, inv, swp)
            out += ([v * i0 for v in a[0:3]] + [jnp.where(low, a[3], b[0]) * swp]
                    + [v * i1 for v in b[1:4]])
        out = spin(out, -1)
        val["bo", c, u] = out
        if u == UNITS - 1:
            rows = [jnp.concatenate([val["bo", c, r // 14][r % 14], val["bo", c, 4 + r // 14][r % 14]], axis=1)
                    for r in range(D // 8)]
            _operands(lambda r: jnp.concatenate(rows[r // 8:r // 8 + 2], axis=0), bo[c % 3])

    def b_out(c, last):
        y = yield from project(wob, 0, bo[c % 3])
        x = xres[c][0] + y
        yield
        if last:
            obuf[:, tok(c)] = x.astype(BF16)
            o_copies[c].start()
        else:
            yield from residual(c, x, an[c])

    def run(stage, c, *args):
        if 0 <= c < NCH:
            flush({a_kv: (a_k, a_v), a_num: (a_q,), a_out: (a_num,), b_scores: (b_q, b_k, b_v),
                   a_q: (b_out,), a_k: (b_out,), a_v: (b_out,),
                   b_q: (a_out,), b_k: (a_out,), b_v: (a_out,)}.get(stage, ()), c)
            half = args[-1] if args and args[-1] in (LEFT, RIGHT) else None
            args = args[:-1] if half else args
            if half == RIGHT:
                gen = val.pop((stage, c))
                gen.send(False)
            else:
                gen = stage(c, *args)
                if gen is not None:
                    next(gen)
                if half == LEFT:
                    val[stage, c], gen = gen, None
                elif stage in (a_q, a_k, a_v, a_out, b_q, b_k, b_v, b_out):
                    gen.send(True)
            if stage not in (a_kv, a_num, a_norm):
                val["short"] = stage is b_scores
                pending[:] = [p for p in pending if next(p[0], True) is None]
            if gen is not None:
                pending.append((gen, stage, c))

    def flush(stages=None, c=None):
        val["short"] = False
        for p in list(pending):
            if stages is None or (p[1] in stages and p[2] == c):
                pending.remove(p)
                for _ in p[0]:
                    pass

    def stretch(*key):
        val["tune"] = TUNING.get(key, DEFAULT)
        return val["tune"][0]

    pending = []
    stretch(0, 0)

    for buf in an + bn + ao + bo:
        for i in (3, 5):
            buf[i, D - KH:KH, :] = jnp.zeros((2 * KH - D, 128), BF16)
    w_copies[1].wait()
    fold = fold_matrices()
    x_copies[0].wait()
    w_copies[0].wait()
    a_norm(0)
    for cp in x_copies[1:3]:
        cp.start()
    transpose(wtmp[0], wraw_a, [7, 8, 9, 10])
    prepare(wa, 2, wtmp[0])
    w_copies[2].wait()
    for cp in w_copies[3:4] + x_copies[3:]:
        cp.start()
    transpose(wtmp[0], wraw_a, [3, 4, 5, 6])
    run(a_v, 0, LEFT)
    fold_into(fold, 1)
    run(a_v, 0, RIGHT)
    run(a_k, 0)
    for cp in x_copies[1:3]:
        cp.wait()
    a_norm(1)
    for c in range(1, NCH):
        if c == 2:
            for cp in w_copies[3:4] + x_copies[3:]:
                cp.wait()
            for cp in w_copies[4:]:
                cp.start()
            transpose(wtmp[0], wraw_a, [0, 1, 2])
        if c == NCH - 3:
            for cp in w_copies[4:]:
                cp.wait()
        norm, ak, aw, kv = (a_norm, c + 1), (a_k, c), (a_v, c), (a_kv, c - 1)
        for stage in ([norm, ak, kv, aw], [ak, norm, kv, aw], [ak, aw, norm, kv], [aw, norm, kv, ak],
                      [aw, kv, ak, norm], [ak, kv, aw, norm])[stretch(0, c) % 6]:
            run(*stage)
        if c == 4:
            fold_into(fold, 0)
        if c == NCH - 3:
            transpose(wtmp[2], woraw_a, range(4))
        if c == NCH - 2:
            prepare(woa, 0, wtmp[2])
            transpose(wtmp[1], wraw_b, [3, 4, 5, 6])
        if c == NCH - 1:
            prepare(wb, 1, wtmp[1])
            transpose(wtmp[1], wraw_b, [0, 1, 2])

    for first in (True, False):
        stretch(2 - first, -1)
        val["first"] = first
        if first:
            run(a_q, 0)
        flush()
        run(a_kv, NCH - 1)
        run(*((a_q, 1) if first else (a_q, 0, RIGHT)))
        flush()
        run(a_num, 0)
        flush()
        run(a_out, 0, LEFT)
        run(a_num, 1)
        run(a_out, 0, RIGHT)
        if first:
            prepare(wb, 0, wtmp[1], DH ** -0.5 * LOG2E)
        run(a_out, 1)
        run(b_k, 0)
        if first:
            transpose(wtmp[1], wraw_b, [7, 8, 9, 10])
        run(b_q, 0)
        if first:
            prepare(wb, 2, wtmp[1])
            transpose(wtmp[3], woraw_b, range(4))
        run(b_v, 0)
        if first:
            prepare(wob, 0, wtmp[3])
        for c in range(NCH + 1):
            bk, bq, bv = ((f, c + 1) for f in (b_k, b_q, b_v))
            aq, nm, ax = ((f, c + 2) for f in (a_q, a_num, a_out))
            bx, ak, aw, kv = (b_out, c - 1, not first), (a_k, c - 1), (a_v, c - 1), (a_kv, c - 1)

            def halves(stage):
                return [[stage + (LEFT,)], [stage + (RIGHT,)]]

            order = stretch(2 - first, c)
            if c == NCH and first:
                fill = [[(a_q, 0, LEFT)], [bx, (a_v, c - 2), (a_kv, c - 2), ak, aw]]
            elif c == NCH:
                fill = [[(b_out, c - 2, True, RIGHT)], [bx]]
            elif c == 0:
                fill = ([[aq]] + halves(bk) + [[bq + (LEFT,), nm], [bq + (RIGHT,)], [ax]] + halves(bv),
                        halves(bk) + [[aq]] + halves(bq) + [[bv + (LEFT,), nm], [bv + (RIGHT,)], [ax]],
                        [[aq]] + halves(bk) + [[bq, nm]] + halves(ax) + halves(bv))[order % 3]
            elif c < NCH - 2:
                fill = ([[[bk], [aq], [bx], [bq, nm], [ak], [aw], [ax], [bv, kv]],
                         [[aq], [bk], [bx, nm], [bq], [aw], [ak], [bv], [ax, kv]],
                         [[bk], [bq], [bx], [aq], [aw], [ak, nm], [bv], [ax, kv]],
                         [[aq], [bk], [bx], [bv, nm], [ak], [ax], [aw], [bq, kv]]] if first else
                        [halves(bk) + [[aq], [bx], [bq, nm], [ax]] + halves(bv),
                         [[aq]] + halves(bk) + [[bx, nm], [bq], [ax]] + halves(bv),
                         [[aq], [bk]] + halves(bx) + [[bq, nm]] + halves(ax) + [[bv]],
                         halves(aq) + [[bx], [bk, nm]] + halves(bq) + [[ax], [bv]]])[order % 4]
            elif first and c == NCH - 2:
                fill = (halves(bk) + [[bx], [bq], [ak], [aw]] + halves(bv),
                        halves(bk) + [[bx]] + halves(bq) + [[ak], [aw], [bv]],
                        halves(bk) + [[bx], [bq]] + halves(aw) + [[ak], [bv]])[order % 3]
            elif first:
                old, nq = (a_kv, c - 2), (a_q, 1)
                fill = (halves(nq) + halves(bx) + [[old]] + halves(ak) + [[]],
                        [[nq], [old]] + halves(bx) + [[], [ak + (LEFT,)], [], [ak + (RIGHT,)]],
                        [[nq + (LEFT,)], [old], [bx + (LEFT,)], [bx + (RIGHT,)], [nq + (RIGHT,)], [],
                         [ak + (LEFT,)], [ak + (RIGHT,)]])[order % 3]
            elif c == NCH - 2:
                fill = halves(bk) + [[], []] + halves(bq) + halves(bv)
            else:
                old = (b_out, c - 2, True)
                fill = [[old + (LEFT,)], [], [old + (RIGHT,)], [], [], [bx + (LEFT,)], [], []]
            for u in range(len(fill)):
                run(b_scores, c, u)
                if (c, u) == (NCH, 0):
                    flush()
                    run(b_pv, NCH - 1, UNITS - 2)
                    val["ticks"] = None
                    b_mix(NCH - 1, UNITS - 1)
                if (c, u) == (NCH, 1):
                    run(b_pv, NCH - 1, UNITS - 1)
                    flush()
                for stage in fill[u]:
                    run(*stage)
                if not any(stage[0] is not a_kv for stage in fill[u]):
                    val["ticks"] = None
                    flush()

    flush()
    for cp in o_copies:
        cp.wait()


@jax.jit
def pallas_interleave_layers__linear_kernel_hedgehog__sliding_block__prompt_kernel(
    A_x: jax.Array,
    A_wqkv: jax.Array,
    A_w_phi: jax.Array,
    A_wo: jax.Array,
    B_x: jax.Array,
    B_wqkv: jax.Array,
    B_wo: jax.Array,
):
    del B_x
    hbm = pl.BlockSpec(memory_space=pltpu.MemorySpace.HBM)
    vmem = pltpu.VMEM
    operands = vmem((7, KH, 128), BF16)
    out = pl.pallas_call(
        _kernel,
        in_specs=[hbm] * 6,
        out_specs=hbm,
        out_shape=jax.ShapeDtypeStruct((D, S), BF16),
        scratch_shapes=[
            [vmem((2, D, T), BF16)] * NCH,
            vmem((D, 3 * D), BF16),
            vmem((D, 3 * D), BF16),
            vmem((D, D), BF16),
            vmem((D, D), BF16),
            vmem((DH, H, DH), BF16),
            vmem((21, 2, MH, 128), BF16),
            vmem((21, 2, MH, 128), BF16),
            vmem((7, 2, MH, 128), BF16),
            vmem((7, 2, MH, 128), BF16),
            [vmem((2, 4 * n * D, 128), BF16) for n in (3, 3, 1, 1)],
            [vmem((8, 2, 128, 128), BF16)] * 2,
            vmem((8, 64, 128), BF16),
            vmem((4, S, 128), BF16),
            vmem((S // 128, H * 32, 128), BF16),
            vmem((2, UNITS, 112, 128), BF16),
            [vmem((8, 2, 128, 128), BF16)] * 2,
            [vmem((8, 2, 64, 128), BF16)] * 2,
            [operands] * 2,
            [operands] * 3,
            vmem((D, S), BF16),
            pltpu.SemaphoreType.DMA((NCH,)),
            pltpu.SemaphoreType.DMA((7,)),
            pltpu.SemaphoreType.DMA((NCH,)),
            pltpu.SemaphoreType.REGULAR((3,)),
            [vmem((2, 32, 128), F32)] * NBUF,
            [vmem((2, 4 * 288, 128), BF16)] * NBUF,
            [vmem((2, 256, 128), F32)] * (4 * NBUF),
            [vmem((2, D, T), F32)] * NCH,
            [operands] * NCH,
            [operands] * 2,
        ],
        compiler_params=pltpu.CompilerParams(vmem_limit_bytes=100 << 20),
    )(A_x[0].T, A_wqkv, A_w_phi.transpose(1, 0, 2), A_wo, B_wqkv, B_wo)
    return out.T[None]
```
